```python
import jax
import jax.numpy as jnp

def _softmax(x, axis=-1):
    return jax.nn.softmax(x, axis=axis)
def _gelu(x):
    return jax.nn.gelu(x, approximate=True)
def _silu(x):
    return jax.nn.silu(x)
def _sigmoid(x):
    return jax.nn.sigmoid(x)
def _layernorm(x, axis=-1, eps=1e-5):
    m = jnp.mean(x, axis=axis, keepdims=True)
    v = jnp.var(x, axis=axis, keepdims=True)
    return (x - m) / jnp.sqrt(v + eps)
def _scatter_add(tgt, idx, src, axis=0):
    return tgt.at[idx].add(src)
def _segment_sum(src, seg, n):
    return jax.ops.segment_sum(src, seg, n)
class _Rng:
    def __init__(self, key):
        self._k = key
    def _next(self):
        self._k, sub = jax.random.split(self._k)
        return sub
    def normal(self, shape):
        return jax.random.normal(self._next(), shape, dtype=jnp.bfloat16)
    def randint(self, lo, hi, shape):
        return jax.random.randint(self._next(), shape, lo, hi, dtype=jnp.int32)
    def uniform(self, shape, lo=0.0, hi=1.0):
        return jax.random.uniform(self._next(), shape, jnp.bfloat16, lo, hi)
    def permutation(self, n):
        return jax.random.permutation(self._next(), n)


kernel_name = 'standalone__gqa_block_cached__near_ridge'

def setup_inputs():
    _rng = _Rng(jax.random.key(int.from_bytes(__import__("os").urandom(4), "little")))
    _w = (lambda a: (lambda t: t.astype(jnp.bfloat16) if jnp.issubdtype(t.dtype, jnp.floating) else t)(jnp.asarray(a)))
    B, Sq, D = 16, 240, 640
    Hq, Hkv, Sk, Dh = 32, 32, 1024, 128
    assert Hq % Hkv == 0, (Hq, Hkv)
    return {
        "x": _w((lambda *s: _rng.normal(s) * 0.05)(B, Sq, D)),
        "k_cache": _w((lambda *s: _rng.normal(s) * 0.05)(B, Hkv, Sk, Dh)),
        "v_cache": _w((lambda *s: _rng.normal(s) * 0.05)(B, Hkv, Sk, Dh)),
        "wq": _w((lambda *s: _rng.normal(s) * 0.05)(D, Hq * Dh) * (D ** -0.5)),
        "wo": _w((lambda *s: _rng.normal(s) * 0.05)(Hq * Dh, D) * ((Hq * Dh) ** -0.5)),
    }

def reference(x, k_cache, v_cache, wq, wo):
    B, Sq, D = x.shape
    Hq, Dh = 32, 128
    Hkv = k_cache.shape[1]
    rep = Hq // Hkv
    q = (lambda x, *d: x.transpose(*d))((x @ wq).reshape(B, Sq, Hq, Dh), 0, 2, 1, 3)
    k = jnp.repeat(k_cache, rep, axis=1)
    v = jnp.repeat(v_cache, rep, axis=1)
    scores = jnp.einsum("bhqd,bhkd->bhqk", q, k) * (Dh ** -0.5)
    p = _softmax(scores, axis=-1)
    o = jnp.einsum("bhqk,bhkd->bhqd", p, v)
    return (lambda x, *d: x.transpose(*d))(o, 0, 2, 1, 3).reshape(B, Sq, Hq * Dh) @ wo
```

```python
import functools
import jax, jax.numpy as jnp
import jax.experimental.pallas as pl
import jax.experimental.pallas.tpu as pltpu

LOG2E = 1.4426950408889634
NT = (((1,), (1,)), ((), ()))
f32, bf16 = jnp.float32, jnp.bfloat16
F = {'XLA_TPU_RESCHEDULE_DMA_DONES': True}

def recip(l):
    r = pl.reciprocal(l, approx=True)
    return r * (2.0 - l * r)

def parse(s):
    n = {"Q": 0, "O": 0}; out = []
    for slot in s.split(","):
        items = []
        for ch in slot:
            items.append((ch, n[ch])); n[ch] += 1
        out.append(items)
    assert n == {"Q": 5, "O": 5} and len(out) == 8
    return out

def _make(sched=",QQO,,QQO,,QO,,OO", rc=48, flags=F, B=16, H=32, R=8, ancj=None):
    Sq, D = 240, 640
    NJ = H // 4; NU = 2 * NJ; NP = B // 2; NG = NP * NU
    R = min(R, NU); AH = R - 1
    assert NU % R == 0
    slots = parse(sched)
    c = (128 ** -0.5) * LOG2E
    def kernel(x_hbm, k_hbm, v_hbm, wq_hbm, wo_hbm, o_hbm, xbuf, kvbuf, wq_ref, wo_ref, q_scr, o_scr, acc_scr, obuf, s_scr, m_scr,
               xsem, ksem, vsem, wqsem, wosem, osem):
        def x_copy(p):
            return pltpu.make_async_copy(x_hbm.at[pl.ds(2 * p, 2)], xbuf.at[p % 2], xsem.at[p % 2 + 1])
        def kv_copy(hbm, w, sem, gi, slot):
            b = 2 * (gi // NU) + gi % 2; j = (gi % NU) // 2
            return pltpu.make_async_copy(hbm.at[b, pl.ds(j * 4, 4)], kvbuf.at[slot, w], sem.at[slot + 1])
        k_copy = functools.partial(kv_copy, k_hbm, 0, ksem)
        v_copy = functools.partial(kv_copy, v_hbm, 1, vsem)
        def blk(j):
            return pl.ds(j * 512 if isinstance(j, int) else pl.multiple_of(j * 512, 512), 512)
        def wq_copy(j):
            return pltpu.make_async_copy(wq_hbm.at[:, blk(j)], wq_ref.at[:, blk(j)], wqsem.at[j + 1])
        def wo_copy(j):
            return pltpu.make_async_copy(wo_hbm.at[blk(j)], wo_ref.at[blk(j)], wosem.at[j + 1])
        def o_copy(b, i):
            return pltpu.make_async_copy(obuf.at[i], o_hbm.at[b], osem.at[i + 1])
        def qdot(xs, bb, j, k):
            return jnp.dot(xbuf[xs, bb, :, k * 128:(k + 1) * 128], wq_ref[k * 128:(k + 1) * 128, blk(j)], preferred_element_type=f32)
        def odot(oc, j, n):
            return jnp.dot(oc, wo_ref[blk(j), n * 128:(n + 1) * 128], preferred_element_type=f32)

        one = pl.program_id(0) + 1
        def s0(i, cc):
            x_copy(0).start()
            wq_copy(0).start()
        jax.lax.fori_loop(0, one, s0, None)
        def s1(u, cc):
            pl.when((u % 2 == 1) & ((u + 1) // 2 < NJ))(lambda: wq_copy((u + 1) // 2).start())
            pl.when((u % 2 == 0) & (u > 0))(lambda: wo_copy(u // 2 - 1).start())
            k_copy(u, u).start()
            v_copy(u, u).start()
        jax.lax.fori_loop(0, one * AH, s1, None)
        o_scr[...] = jnp.zeros_like(o_scr)
        acc_scr[...] = jnp.zeros_like(acc_scr)
        x_copy(0).wait()
        wq_copy(0).wait()
        qq = qdot(0, 0, 0, 0)
        for k in range(1, 5): qq = qq + qdot(0, 0, 0, k)
        qq = (qq * c).astype(bf16)
        q_scr[...] = qq
        k_copy(0, 0).wait()
        def carry_s(sv):
            s_scr[...] = sv
            m_scr[...] = jnp.broadcast_to(jnp.max(sv, axis=-1, keepdims=True), m_scr.shape)
        carry_s(jax.lax.dot_general(qq[:, :128], kvbuf[0, 0, 0], NT, preferred_element_type=f32))

        U = 8
        def body(t, carry):
            p, half = t // 2, t % 2
            first = t < 2
            acc = {0: [None] * 5, 1: [None] * 5}
            qpart, q, o, ocat = {}, {0: q_scr}, {}, {}
            def Q(u, k):
                if u < U:
                    xs, j = p % 2, half * (U // 2) + u // 2
                    if k == 0 and u % 2 == 0: pl.when(first)(lambda: wq_copy(j).wait())
                else:
                    xs, j = (p + half) % 2, (1 - half) * (U // 2)
                    if k == 0:
                        pl.when((half == 1) & (p + 1 < NP))(lambda: x_copy(p + 1).wait())
                        pl.when(t == 0)(lambda: wq_copy(U // 2).wait())
                d = qdot(xs, u % 2, j, k)
                qpart[u] = d if k == 0 else qpart[u] + d
                if k == 4:
                    qv = (qpart.pop(u) * c).astype(bf16)
                    q[u] = qv
                    if u == U: q_scr[...] = qv
                    if u == 1: pl.when((half == 0) & (p + 1 < NP))(lambda: x_copy(p + 1).start())
            def O(u, n):
                cs = slice(n * 128, (n + 1) * 128)
                a = acc[u % 2]
                if u < 0:
                    if n == 0: pl.when((half == 1) & (t > 1))(lambda: o_copy(2 * p - 1, 1).wait())
                    a[n] = acc_scr[1, :, cs] + odot(o_scr[...], (1 - half) * (U // 2) + U // 2 - 1, n)
                    obuf[1, :, cs] = a[n].astype(bf16)
                    if n == 4: pl.when((half == 0) & (t > 0))(lambda: o_copy(2 * p - 1, 1).start())
                    return
                j = half * (U // 2) + u // 2
                if n == 0:
                    ocat[u] = jnp.concatenate([o.pop(4 * u + i) for i in range(4)], axis=1)
                    if u % 2 == 0: pl.when(first)(lambda: wo_copy(j).wait())
                d = odot(ocat[u], j, n)
                if u == 0: a[n] = jnp.where(half == 0, 0.0, acc_scr[0, :, cs]) + d
                elif u == 1: a[n] = jnp.where(half == 0, 0.0, a[n]) + d
                else: a[n] = a[n] + d
                if u >= U - 3: acc_scr[u % 2, :, cs] = a[n]
                if u == U - 2:
                    if n == 0: pl.when((half == 0) & (t > 0))(lambda: o_copy(2 * p - 2, 0).wait())
                    obuf[0, :, cs] = a[n].astype(bf16)
                    if n == 4: pl.when(half == 1)(lambda: o_copy(2 * p, 0).start())
            def QK(h):
                u = h // 4
                if h % 4 == 0:
                    if u < U: k_copy(t * U + u, u % R).wait()
                    else: pl.when(t + 1 < 2 * NP)(lambda: k_copy(t * U + u, u % R).wait())
                return jax.lax.dot_general(q[u][:, (h % 4) * 128:(h % 4 + 1) * 128], kvbuf[u % R, 0, h % 4], NT, preferred_element_type=f32)
            def SM(s):
                ps, rs = [], []
                for r0 in range(0, 240, rc):
                    if s is None:
                        sc = s_scr[r0:r0 + rc]
                        m = jnp.tile(m_scr[r0:r0 + rc], (1, 8))
                    else:
                        sc = s[r0:r0 + rc]
                        m = jnp.max(sc, axis=-1, keepdims=True)
                    if ancj is None:
                        pp = jnp.exp2(sc - m)
                        l = jnp.sum(pp, axis=-1, keepdims=True)
                        pp = pp.astype(bf16)
                    else:
                        pl_ = []; run = None
                        for jj in range(8):
                            e = jnp.exp2(sc[:, jj * 128:(jj + 1) * 128] - m[:, :128])
                            run = e if run is None else run + e
                            if jj in ancj: e = jnp.minimum(e, run)
                            pl_.append(e.astype(bf16))
                        l = jnp.sum(run, axis=-1, keepdims=True)
                        pp = jnp.concatenate(pl_, axis=1)
                    ps.append(pp); rs.append(recip(l))
                cat = lambda a: jnp.concatenate(a, axis=0) if len(a) > 1 else a[0]
                return cat(ps), cat(rs)
            def refill(u):
                a = u + AH
                gi = t * U + a
                if a % 2 == 1: pl.when((gi + 1) // 2 < NJ)(lambda: wq_copy((gi + 1) // 2).start())
                else: pl.when(gi // 2 - 1 < NJ)(lambda: wo_copy(gi // 2 - 1).start())
                @pl.when(gi < NG)
                def _():
                    k_copy(gi, a % R).start()
                    v_copy(gi, a % R).start()
            def PV(h, pp, r):
                u = h // 4
                if h % 4 == 0:
                    v_copy(t * U + u, u % R).wait()
                    refill(u)
                o[h] = (jnp.dot(pp, kvbuf[u % R, 1, h % 4], preferred_element_type=f32) * r).astype(bf16)
            s = {0: None}
            G = 4 * U
            for h in range(G):
                u, i = divmod(h, 4)
                def fill(items):
                    for tt, n in items:
                        if tt == "Q": Q(u + 1, n)
                        else: O(u - 1, n)
                s[h + 1] = QK(h + 1)
                if h + 1 == G: carry_s(s[G])
                fill(slots[2 * i])
                pp, r = SM(s.pop(h))
                PV(h, pp, r)
                fill(slots[2 * i + 1])
            o_scr[...] = jnp.concatenate([o.pop(G - 4 + i) for i in range(4)], axis=1)
        jax.lax.fori_loop(0, 2 * NP, body, None)
        for n in range(5):
            cs = slice(n * 128, (n + 1) * 128)
            obuf[1, :, cs] = (acc_scr[1, :, cs] + odot(o_scr[...], NJ - 1, n)).astype(bf16)
        o_copy(2 * NP - 1, 1).start()
        o_copy(2 * NP - 2, 0).wait()
        o_copy(2 * NP - 1, 1).wait()

    def fn(x, k, v, wq, wo):
        any_spec = pl.BlockSpec(memory_space=pl.ANY)
        return pl.pallas_call(
            kernel,
            grid=(1,),
            in_specs=[any_spec] * 5,
            out_specs=any_spec,
            out_shape=jax.ShapeDtypeStruct((B, Sq, D), x.dtype),
            scratch_shapes=[pltpu.VMEM((2, 2, Sq, D), bf16),
                            pltpu.VMEM((R, 2, 4, 1024, 128), bf16),
                            pltpu.VMEM(wq.shape, bf16), pltpu.VMEM(wo.shape, bf16),
                            pltpu.VMEM((Sq, 512), bf16), pltpu.VMEM((Sq, 512), bf16), pltpu.VMEM((2, Sq, D), f32),
                            pltpu.VMEM((2, Sq, D), bf16), pltpu.VMEM((Sq, 1024), f32), pltpu.VMEM((Sq, 128), f32),
                            pltpu.SemaphoreType.DMA((3,)),
                            pltpu.SemaphoreType.DMA((R + 1,)), pltpu.SemaphoreType.DMA((R + 1,)),
                            pltpu.SemaphoreType.DMA((NJ + 1,)), pltpu.SemaphoreType.DMA((NJ + 1,)),
                            pltpu.SemaphoreType.DMA((3,))],
            compiler_params=pltpu.CompilerParams(
                dimension_semantics=("arbitrary",), flags=flags, disable_bounds_checks=True,
                vmem_limit_bytes=100 * 1024 * 1024),
        )(x, k, v, wq, wo)
    return fn


@jax.jit
def pallas_standalone__gqa_block_cached__near_ridge_kernel(x, k_cache, v_cache, wq, wo):
    return _make()(x, k_cache, v_cache, wq, wo)
```

```python
import functools

import jax
import jax.numpy as jnp
import jax.experimental.pallas as pl
import jax.experimental.pallas.tpu as pltpu

LOG2E = 1.4426950408889634
NT = (((1,), (1,)), ((), ()))
f32, bf16 = jnp.float32, jnp.bfloat16

U = 8
R = 8
AHEAD = 4
NFINE = 2


def _fillers(spec):
    count = {"Q": 0, "O": 0}
    out = []
    for slot in spec.split(","):
        items = []
        for kind in slot:
            items.append((kind, count[kind]))
            count[kind] += 1
        out.append(items)
    assert count == {"Q": 5, "O": 5} and len(out) == 4
    return out


FILL_FIRST = _fillers("QQQO,Q,QO,OOO")
FILL_MID = _fillers("QQ,QQO,QOO,OO")
FILL_LAST = _fillers("QQO,QQO,Q,OOO")


def _recip(l):
    r = pl.reciprocal(l, approx=True)
    return r * (2.0 - l * r)


@jax.jit
def pallas_standalone__gqa_block_cached__near_ridge_kernel(
    x: jax.Array,
    k_cache: jax.Array,
    v_cache: jax.Array,
    wq: jax.Array,
    wo: jax.Array,
):
    B, Sq, D = x.shape
    _, H, Sk, Dh = k_cache.shape
    assert (D, H, Sk, Dh) == (640, 32, 1024, 128) and wq.shape == (D, H * Dh)
    assert B % 2 == 0 and Sq % 48 == 0
    NJ = H // 4
    NU = 2 * NJ
    NP = B // 2
    NG = NP * NU
    RC = 48
    q_scale = Dh ** -0.5 * LOG2E

    def heads_per_copy(slot):
        return 2 if slot < NFINE else 4

    def kernel(x_hbm, k_hbm, v_hbm, wq_hbm, wo_hbm, o_hbm,
               xbuf, kvbuf, wq_ref, wo_ref, q_scr, o_scr, acc_scr, obuf, s_scr, m_scr,
               xsem, ksem, vsem, wqsem, wosem, osem, fsem):

        def x_copy(p, i):
            return pltpu.make_async_copy(x_hbm.at[2 * p + i], xbuf.at[p % 2, i], xsem.at[i + 1])

        def kv_copy(hbm, w, sem, gi, slot, cc, n=None):
            b = 2 * (gi // NU) + gi % 2
            j = (gi % NU) // 2
            n = n or heads_per_copy(slot)
            return pltpu.make_async_copy(
                hbm.at[b, pl.ds(j * 4 + cc * n, n)],
                kvbuf.at[slot, w, pl.ds(cc * n, n)],
                sem.at[slot * 2 + cc + 1])

        k_copy = functools.partial(kv_copy, k_hbm, 0, ksem)
        v_copy = functools.partial(kv_copy, v_hbm, 1, vsem)

        def blk(j):
            return pl.ds(j * 512 if isinstance(j, int) else pl.multiple_of(j * 512, 512), 512)

        def wq_copy(j):
            return pltpu.make_async_copy(wq_hbm.at[:, blk(j)], wq_ref.at[:, blk(j)], wqsem.at[j + 1])

        def wo_copy(j):
            return pltpu.make_async_copy(wo_hbm.at[blk(j)], wo_ref.at[blk(j)], wosem.at[j + 1])

        def o_copy(b, i):
            return pltpu.make_async_copy(obuf.at[i], o_hbm.at[b], osem.at[i + 1])

        def last_copy(n):
            cs = pl.ds(n * 128, 128)
            return pltpu.make_async_copy(obuf.at[1, :, cs], o_hbm.at[B - 1, :, cs], fsem.at[n])

        def qdot(xs, bb, j, k):
            ks = slice(k * 128, (k + 1) * 128)
            return jnp.dot(xbuf[xs, bb, :, ks], wq_ref[ks, blk(j)], preferred_element_type=f32)

        def odot(oc, j, n):
            return jnp.dot(oc, wo_ref[blk(j), n * 128:(n + 1) * 128], preferred_element_type=f32)

        def carry_scores(sv):
            s_scr[...] = sv
            m_scr[...] = jnp.broadcast_to(jnp.max(sv, axis=-1, keepdims=True), m_scr.shape)

        one = pl.program_id(0) + 1

        def start_first(i, carry):
            x_copy(0, 0).start()
            wq_copy(0).start()

        jax.lax.fori_loop(0, one, start_first, None)

        def start_units(n, u0, i, carry):
            u, cc = u0 + i // (4 // n), i % (4 // n)
            k_copy(u, u, cc, n).start()
            v_copy(u, u, cc, n).start()
            if u0 == 0:
                pl.when(i == 0)(lambda: x_copy(0, 1).start())
            pl.when((u % 2 == 1) & (cc == 0))(lambda: wq_copy((u + 1) // 2).start())
            pl.when((u % 2 == 1) & (cc == 0))(lambda: wo_copy((u - 1) // 2).start())

        jax.lax.fori_loop(0, one * NFINE * 2, functools.partial(start_units, 2, 0), None)
        jax.lax.fori_loop(0, one * (AHEAD - NFINE), functools.partial(start_units, 4, NFINE), None)

        o_scr[...] = jnp.zeros(o_scr.shape, bf16)
        acc_scr[...] = jnp.zeros_like(acc_scr)
        wo_ref[blk(NJ - 1)] = jnp.zeros((512, D), bf16)
        x_copy(0, 0).wait()
        wq_copy(0).wait()
        q0 = qdot(0, 0, 0, 0)
        for k in range(1, 5):
            q0 = q0 + qdot(0, 0, 0, k)
        q0 = (q0 * q_scale).astype(bf16)
        q_scr[...] = q0
        k_copy(0, 0, 0).wait()
        carry_scores(jax.lax.dot_general(q0[:, :128], kvbuf[0, 0, 0], NT, preferred_element_type=f32))

        def body(t, carry):
            p, half = t // 2, t % 2
            first = t < 2
            acc = {0: [None] * 5, 1: [None] * 5}
            qtail, q, o, ocat = {}, {}, {}, {}

            def q_slice(u, k):
                if u < U:
                    xs, j = p % 2, half * (U // 2) + u // 2
                    if k == 0 and u % 2 == 0:
                        pl.when(first)(lambda: wq_copy(j).wait())
                    if k == 0 and u == 1:
                        pl.when(half == 0)(lambda: x_copy(p, 1).wait())
                else:
                    xs, j = (p + half) % 2, (1 - half) * (U // 2)
                    if k == 0:
                        pl.when((half == 1) & (p + 1 < NP))(lambda: x_copy(p + 1, 0).wait())
                        pl.when(t == 0)(lambda: wq_copy(U // 2).wait())
                if k == 0:
                    qtail[u] = qdot(xs, u % 2, j, 4)
                else:
                    i = k - 1
                    w = wq_ref[0:512, pl.ds(pl.multiple_of(j * 512 + i * 128, 128), 128)]
                    d = jnp.dot(xbuf[xs, u % 2, :, 0:512], w, preferred_element_type=f32)
                    qv = ((d + qtail[u][:, i * 128:(i + 1) * 128]) * q_scale).astype(bf16)
                    q[4 * u + i] = qv
                    if u == U:
                        q_scr[:, i * 128:(i + 1) * 128] = qv
                if k == 4 and u == 1:
                    @pl.when((half == 1) & (p + 1 < NP))
                    def _():
                        x_copy(p + 1, 0).start()
                        x_copy(p + 1, 1).start()

            def o_slice(u, n):
                cs = slice(n * 128, (n + 1) * 128)
                a = acc[u % 2]
                if u < 0:
                    if n == 0:
                        pl.when((half == 1) & (t > 1))(lambda: o_copy(2 * p - 1, 1).wait())
                    a[n] = acc_scr[1, :, cs] + odot(o_scr[...], (1 - half) * (U // 2) + U // 2 - 1, n)
                    obuf[1, :, cs] = a[n].astype(bf16)
                    if n == 4:
                        pl.when((half == 0) & (t > 0))(lambda: o_copy(2 * p - 1, 1).start())
                    return
                j = half * (U // 2) + u // 2
                if n == 0:
                    heads = [o.pop(4 * u + i) for i in range(4)]
                    ocat[u] = jnp.concatenate(heads, axis=1).astype(bf16)
                    if u % 2 == 0:
                        pl.when(first)(lambda: wo_copy(j).wait())
                d = odot(ocat[u], j, n)
                if u == 0:
                    a[n] = jnp.where(half == 0, 0.0, acc_scr[0, :, cs]) + d
                elif u == 1:
                    a[n] = jnp.where(half == 0, 0.0, a[n]) + d
                else:
                    a[n] = a[n] + d
                if u >= U - 3:
                    acc_scr[u % 2, :, cs] = a[n]
                if u == U - 2:
                    if n == 0:
                        pl.when((half == 0) & (t > 0))(lambda: o_copy(2 * p - 2, 0).wait())
                    obuf[0, :, cs] = a[n].astype(bf16)
                    if n == 4:
                        pl.when(half == 1)(lambda: o_copy(2 * p, 0).start())

            def scores(h):
                u = h // 4
                n = heads_per_copy(u % R)
                if h % n == 0:
                    cc = (h % 4) // n
                    if u < U:
                        k_copy(t * U + u, u % R, cc).wait()
                    else:
                        pl.when(t + 1 < 2 * NP)(lambda: k_copy(t * U + u, u % R, cc).wait())
                qh = q_scr[:, h * 128:(h + 1) * 128] if h < 4 else q.pop(h)
                return jax.lax.dot_general(qh, kvbuf[u % R, 0, h % 4], NT, preferred_element_type=f32)

            def softmax(s):
                ps, rs = [], []
                for r0 in range(0, Sq, RC):
                    if s is None:
                        sc = s_scr[r0:r0 + RC]
                        m = m_scr[r0:r0 + RC]
                    else:
                        sc = s[r0:r0 + RC]
                        m = jnp.max(sc, axis=-1, keepdims=True)
                    es, run = [], None
                    for c in range(Sk // 128):
                        e = jnp.exp2(sc[:, c * 128:(c + 1) * 128] - m)
                        run = e if run is None else run + e
                        if c % 4 == 3:
                            e = jnp.minimum(e, run)
                        es.append(e)
                    ps.append(jnp.concatenate(es, axis=1))
                    rs.append(_recip(jnp.sum(run, axis=-1, keepdims=True)))
                return jnp.concatenate(ps, axis=0).astype(bf16), jnp.concatenate(rs, axis=0)

            def refill(u):
                a = u + AHEAD
                gi = t * U + a

                @pl.when(gi < NG)
                def _():
                    for cc in range(4 // heads_per_copy(a % R)):
                        k_copy(gi, a % R, cc).start()
                        v_copy(gi, a % R, cc).start()

                if a % 2 == 1:
                    pl.when((gi + 1) // 2 < NJ)(lambda: wq_copy((gi + 1) // 2).start())
                    pl.when((gi - 1) // 2 < NJ)(lambda: wo_copy((gi - 1) // 2).start())

            def weighted_values(h, e, r):
                u = h // 4
                n = heads_per_copy(u % R)
                if h % n == 0:
                    v_copy(t * U + u, u % R, (h % 4) // n).wait()
                if h % 4 == 0:
                    refill(u)
                o[h] = jnp.dot(e, kvbuf[u % R, 1, h % 4], preferred_element_type=f32) * r

            G = 4 * U
            s = {0: None}
            for h in range(G):
                u, i = divmod(h, 4)
                s[h + 1] = scores(h + 1)
                if h + 1 == G:
                    carry_scores(s[G])
                weighted_values(h, *softmax(s.pop(h)))
                fill = FILL_LAST if u == U - 1 else FILL_FIRST if u == 0 else FILL_MID
                for kind, n in fill[i]:
                    if kind == "Q":
                        q_slice(u + 1, n)
                    else:
                        o_slice(u - 1, n)
            for i in range(4):
                o_scr[:, i * 128:(i + 1) * 128] = o.pop(G - 4 + i).astype(bf16)

        jax.lax.fori_loop(0, 2 * NP, body, None)

        for n in range(5):
            cs = slice(n * 128, (n + 1) * 128)
            obuf[1, :, cs] = (acc_scr[1, :, cs] + odot(o_scr[...], NJ - 1, n)).astype(bf16)
            last_copy(n).start()
        o_copy(B - 2, 0).wait()
        for n in range(5):
            last_copy(n).wait()

    any_spec = pl.BlockSpec(memory_space=pl.ANY)
    return pl.pallas_call(
        kernel,
        grid=(1,),
        in_specs=[any_spec] * 5,
        out_specs=any_spec,
        out_shape=jax.ShapeDtypeStruct((B, Sq, D), x.dtype),
        scratch_shapes=[
            pltpu.VMEM((2, 2, Sq, D), bf16),
            pltpu.VMEM((R, 2, 4, Sk, Dh), bf16),
            pltpu.VMEM((D, H * Dh), bf16),
            pltpu.VMEM((H * Dh, D), bf16),
            pltpu.VMEM((Sq, 4 * Dh), bf16),
            pltpu.VMEM((Sq, 4 * Dh), bf16),
            pltpu.VMEM((2, Sq, D), f32),
            pltpu.VMEM((2, Sq, D), bf16),
            pltpu.VMEM((Sq, Sk), f32),
            pltpu.VMEM((Sq, 128), f32),
            pltpu.SemaphoreType.DMA((3,)),
            pltpu.SemaphoreType.DMA((2 * R + 1,)),
            pltpu.SemaphoreType.DMA((2 * R + 1,)),
            pltpu.SemaphoreType.DMA((NJ + 1,)),
            pltpu.SemaphoreType.DMA((NJ + 1,)),
            pltpu.SemaphoreType.DMA((3,)),
            pltpu.SemaphoreType.DMA((5,)),
        ],
        compiler_params=pltpu.CompilerParams(
            dimension_semantics=("arbitrary",),
            flags={"XLA_TPU_RESCHEDULE_DMA_DONES": True},
            disable_bounds_checks=True,
            vmem_limit_bytes=64 * 1024 * 1024,
        ),
    )(x, k_cache, v_cache, wq, wo)
```
